```python
import jax
import jax.numpy as jnp

def _softmax(x, axis=-1):
    return jax.nn.softmax(x, axis=axis)
def _gelu(x):
    return jax.nn.gelu(x, approximate=True)
def _silu(x):
    return jax.nn.silu(x)
def _sigmoid(x):
    return jax.nn.sigmoid(x)
def _layernorm(x, axis=-1, eps=1e-5):
    m = jnp.mean(x, axis=axis, keepdims=True)
    v = jnp.var(x, axis=axis, keepdims=True)
    return (x - m) / jnp.sqrt(v + eps)
def _scatter_add(tgt, idx, src, axis=0):
    return tgt.at[idx].add(src)
def _segment_sum(src, seg, n):
    return jax.ops.segment_sum(src, seg, n)
class _Rng:
    def __init__(self, key):
        self._k = key
    def _next(self):
        self._k, sub = jax.random.split(self._k)
        return sub
    def normal(self, shape):
        return jax.random.normal(self._next(), shape, dtype=jnp.bfloat16)
    def randint(self, lo, hi, shape):
        return jax.random.randint(self._next(), shape, lo, hi, dtype=jnp.int32)
    def uniform(self, shape, lo=0.0, hi=1.0):
        return jax.random.uniform(self._next(), shape, jnp.bfloat16, lo, hi)
    def permutation(self, n):
        return jax.random.permutation(self._next(), n)


kernel_name = 'recurrent_scan__compressed_kv_cla__dense_activation_silu__decode'

def setup_inputs():
    _rng = _Rng(jax.random.key(int.from_bytes(__import__("os").urandom(4), "little")))
    _w = (lambda a: (lambda t: t.astype(jnp.bfloat16) if jnp.issubdtype(t.dtype, jnp.floating) else t)(jnp.asarray(a)))
    def _A_setup():
        B, H, Sq, Sk, D, M = 1, 32, 1, 32768, 128, 512
        Dc = 4 * D
        return {
            "x": _w((lambda *s: _rng.normal(s) * 0.05)(B, Sq, M)),
            "c_kv": _w((lambda *s: _rng.normal(s) * 0.05)(B, Sk, Dc)),
            "w_q": _w((lambda *s: _rng.normal(s) * 0.05)(M, H, D) * (M ** -0.5)),
            "w_uk": _w((lambda *s: _rng.normal(s) * 0.05)(Dc, H, D) * (Dc ** -0.5)),
            "w_uv": _w((lambda *s: _rng.normal(s) * 0.05)(Dc, H, D) * (Dc ** -0.5)),
            "w_o": _w((lambda *s: _rng.normal(s) * 0.05)(H, D, M) * ((H * D) ** -0.5)),
        }
    _A_in = _A_setup()

    def _B_setup():
        B, S, D, F = 1, 1, 512, 1376
        return {
            "x": _w((lambda *s: _rng.normal(s) * 0.05)(B, S, D)),
            "w1": _w((lambda *s: _rng.normal(s) * 0.05)(D, F) * (D ** -0.5)),
            "w2": _w((lambda *s: _rng.normal(s) * 0.05)(F, D) * (F ** -0.5)),
        }
    _B_in = _B_setup()

    return {
        "A_x": _A_in["x"],
        "A_c_kv": _A_in["c_kv"],
        "A_w_q": _A_in["w_q"],
        "A_w_uk": _A_in["w_uk"],
        "A_w_uv": _A_in["w_uv"],
        "A_w_o": _A_in["w_o"],
        "B_x": _B_in["x"],
        "B_w1": _B_in["w1"],
        "B_w2": _B_in["w2"],
    }

def reference(A_x, A_c_kv, A_w_q, A_w_uk, A_w_uv, A_w_o, B_x, B_w1, B_w2):
    def _A_ref(x, c_kv, w_q, w_uk, w_uv, w_o):
        B, Sq, M = x.shape[0], x.shape[1], x.shape[2]
        Sk = c_kv.shape[1]
        H, D = w_q.shape[1], w_q.shape[2]
        q = jnp.einsum("bqm,mhd->bhqd", x, w_q)
        k = jnp.einsum("bkc,chd->bhkd", c_kv, w_uk)
        v = jnp.einsum("bkc,chd->bhkd", c_kv, w_uv)
        scores = jnp.einsum("bhqd,bhkd->bhqk", q, k) * (D ** -0.5)
        off = Sk - Sq
        qi = jnp.arange(Sq)[:, None]
        kj = jnp.arange(Sk)[None, :]
        cmask = kj <= (qi + off)
        scores = jnp.where(cmask[None, None], scores, -1e9)
        p = _softmax(scores, axis=-1)
        ctx = jnp.einsum("bhqk,bhkd->bhqd", p, v)
        return jnp.einsum("bhqd,hdm->bqm", ctx, w_o)

    def _B_ref(x, w1, w2):
        h = jnp.einsum("bsd,df->bsf", x, w1)
        h = _silu(h)
        out = jnp.einsum("bsf,fd->bsd", h, w2)
        return out

    x = A_x
    xn = _layernorm(x, axis=-1)
    s = _A_ref(xn, A_c_kv, A_w_q, A_w_uk, A_w_uv, A_w_o)
    g = _silu(_B_ref(xn, B_w1, B_w2))
    return x + s * g
```

```python
import jax
import jax.numpy as jnp
from jax import lax
from jax.experimental import pallas as pl
from jax.experimental.pallas import tpu as pltpu

F32 = jnp.float32
BF16 = jnp.bfloat16
I32 = jnp.int32
_NN = (((1,), (0,)), ((), ()))
_NT = (((1,), (1,)), ((), ()))
LANES = 128

_KEY_BLOCK = 1024
_CKV_PIECES = (16, 9, 5, 2)
_WO_PIECES = (16, 8, 4, 2, 1, 1)
_WO_GROUP = 4
_Q_UNROLL = 8


def _dot(a, b, dims=_NN):
    return lax.dot_general(a, b, dims, preferred_element_type=F32)


def _pieces(sizes):
    out, start = [], 0
    for n in sizes:
        out.append((start, n))
        start += n
    return out


def _split(total, sizes):
    return tuple(sizes) if sum(sizes) == total else (total,)


def _kernel(x_h, c_h, wq_h, wk_h, wv_h, wo_h, w1t_h, w2_h, o_ref,
            x_v, c_v, wq_v, wk_v, wv_v, wo_v, w1t_v, w2_v,
            xn_v, xn_s, qa_v, y_v, lhs_v, sems, sem_xn):
    M, H, D = wq_h.shape
    DC = wk_h.shape[0]
    SK = c_h.shape[1]
    BK = _KEY_BLOCK
    c_pieces = _pieces(_split(SK // BK, _CKV_PIECES))
    wo_pieces = _pieces(_split(H, _WO_PIECES))
    G = LANES // H

    copies = [(x_h, x_v), (w1t_h, w1t_v), (w2_h, w2_v), (wq_h, wq_v), (wk_h, wk_v)]
    copies += [(c_h.at[0, pl.ds(s * BK, n * BK)], c_v.at[pl.ds(s * BK, n * BK)])
               for s, n in c_pieces]
    copies += [(wv_h, wv_v)]
    copies += [(wo_h.at[pl.ds(s, n)], wo_v.at[pl.ds(s, n)]) for s, n in wo_pieces]
    dmas = [pltpu.make_async_copy(src, dst, sems.at[i]) for i, (src, dst) in enumerate(copies)]
    for dma in dmas:
        dma.start()
    stream = iter(dmas)

    def wait_next():
        next(stream).wait()

    wait_next()
    x = x_v[0].astype(F32)
    xc = x - jnp.mean(x, axis=-1, keepdims=True)
    var = jnp.mean(xc * xc, axis=-1, keepdims=True)
    xn = xc / jnp.sqrt(var + 1e-5)
    xn_v[...] = xn
    xn_copy = pltpu.make_async_copy(xn_v, xn_s, sem_xn)
    xn_copy.start()

    xb = jnp.broadcast_to(xn, (16, M)).astype(BF16)
    wait_next()
    h1 = _dot(xb, w1t_v[...], _NT)
    h1 = h1 * jax.nn.sigmoid(h1)
    wait_next()
    ff = _dot(h1.astype(BF16), w2_v[...])[0:1]
    gate = ff * jax.nn.sigmoid(ff)

    xn_copy.wait()
    wait_next()

    def q_step(j, acc):
        acc = list(acc)
        for u in range(_Q_UNROLL):
            m = j * _Q_UNROLL + u
            acc[u % 2] = acc[u % 2] + wq_v[m].astype(F32) * xn_s[0, m]
        return tuple(acc)

    zero = jnp.zeros((H, D), F32)
    qa, qb = lax.fori_loop(0, M // _Q_UNROLL, q_step, (zero, zero))
    q = (qa + qb).astype(BF16)

    row = lax.broadcasted_iota(I32, (H, LANES), 0)
    lane = lax.broadcasted_iota(I32, (H, LANES), 1)
    wait_next()
    pick = (lane % G) * H + row

    def qabs_step(t, carry):
        c0 = pl.multiple_of(t * LANES, LANES)
        r = _dot(q, wk_v[pl.ds(c0, LANES)].reshape(LANES * H, D), _NT)
        out = jnp.zeros((H, LANES), F32)
        for u in range(LANES // G):
            g = jnp.take_along_axis(r[:, u * LANES:(u + 1) * LANES], pick, axis=1)
            out = jnp.where(lane // G == u, g, out)
        qa_v[:, pl.ds(c0, LANES)] = (out * (D ** -0.5)).astype(BF16)
        return carry

    lax.fori_loop(0, DC // LANES, qabs_step, 0)

    def attend(block, carry):
        m_run, l_run, acc = carry
        cb = c_v[pl.ds(pl.multiple_of(block * BK, BK), BK), :]
        s = _dot(qa_v[...], cb, _NT)
        m_new = jnp.maximum(m_run, jnp.max(s, axis=1, keepdims=True))
        alpha = jnp.exp(m_run - m_new)
        p = jnp.exp(s - m_new)
        l_run = alpha * l_run + jnp.sum(p, axis=1, keepdims=True)
        acc = alpha * acc + _dot(p.astype(BF16), cb)
        return m_new, l_run, acc

    carry = (jnp.full((H, 1), -1e30, F32), jnp.zeros((H, 1), F32), jnp.zeros((H, DC), F32))
    for s0, n in c_pieces:
        wait_next()
        carry = lax.fori_loop(s0, s0 + n, attend, carry)
    _, l_run, acc = carry
    y_v[...] = acc / l_run

    spread = lane // H
    diag = (lane % H) == row
    wait_next()

    def ctx_step(t, ctx):
        c0 = pl.multiple_of(t * LANES, LANES)
        yt = y_v[:, pl.ds(c0, LANES)]
        parts = []
        for u in range(LANES // G):
            g = jnp.take_along_axis(yt, G * u + spread, axis=1)
            parts.append(jnp.where(diag, g, 0.0).astype(BF16))
        s = jnp.concatenate(parts, axis=1)
        return ctx + _dot(s, wv_v[pl.ds(c0, LANES)].reshape(LANES * H, D))

    ctx = lax.fori_loop(0, DC // LANES, ctx_step, zero)

    for h in range(H):
        lhs_v[:, h * D:(h + 1) * D] = jnp.broadcast_to(ctx[h:h + 1], (16, D)).astype(BF16)

    def heads(h0, n):
        return _dot(lhs_v[:, pl.ds(pl.multiple_of(h0 * D, D), n * D)],
                    wo_v[pl.ds(h0, n)].reshape(n * D, M))

    o = jnp.zeros((16, M), F32)
    U = _WO_GROUP
    for s0, n in wo_pieces:
        wait_next()
        if n // U > 1:
            o = lax.fori_loop(0, n // U, lambda j, o, s0=s0: o + heads(s0 + j * U, U), o)
        elif n // U == 1:
            o = o + heads(s0, U)
        if n % U:
            o = o + heads(s0 + n // U * U, n % U)
    o_ref[0] = (x + o[0:1] * gate).astype(o_ref.dtype)


@jax.jit
def pallas_recurrent_scan__compressed_kv_cla__dense_activation_silu__decode_kernel(
    A_x: jax.Array,
    A_c_kv: jax.Array,
    A_w_q: jax.Array,
    A_w_uk: jax.Array,
    A_w_uv: jax.Array,
    A_w_o: jax.Array,
    B_x: jax.Array,
    B_w1: jax.Array,
    B_w2: jax.Array,
):
    del B_x
    B, Sq, M = A_x.shape
    _, SK, DC = A_c_kv.shape
    _, H, D = A_w_q.shape
    FF = B_w1.shape[1]
    assert B == 1 and Sq == 1 and D == LANES and LANES % H == 0 and DC % LANES == 0
    assert SK % _KEY_BLOCK == 0 and M % _Q_UNROLL == 0
    n_dma = 6 + len(_split(SK // _KEY_BLOCK, _CKV_PIECES)) + len(_split(H, _WO_PIECES))

    return pl.pallas_call(
        _kernel,
        out_shape=jax.ShapeDtypeStruct(A_x.shape, A_x.dtype),
        in_specs=[pl.BlockSpec(memory_space=pl.ANY)] * 8,
        out_specs=pl.BlockSpec(memory_space=pltpu.VMEM),
        scratch_shapes=[
            pltpu.VMEM((B, Sq, M), A_x.dtype),
            pltpu.VMEM((SK, DC), A_c_kv.dtype),
            pltpu.VMEM(A_w_q.shape, A_w_q.dtype),
            pltpu.VMEM(A_w_uk.shape, A_w_uk.dtype),
            pltpu.VMEM(A_w_uv.shape, A_w_uv.dtype),
            pltpu.VMEM(A_w_o.shape, A_w_o.dtype),
            pltpu.VMEM((FF, M), B_w1.dtype),
            pltpu.VMEM((FF, M), B_w2.dtype),
            pltpu.VMEM((1, M), F32),
            pltpu.SMEM((1, M), F32),
            pltpu.VMEM((H, DC), BF16),
            pltpu.VMEM((H, DC), F32),
            pltpu.VMEM((16, H * D), BF16),
            pltpu.SemaphoreType.DMA((n_dma,)),
            pltpu.SemaphoreType.DMA(()),
        ],
        compiler_params=pltpu.CompilerParams(vmem_limit_bytes=100 * 1024 * 1024),
    )(A_x, A_c_kv, A_w_q, A_w_uk, A_w_uv, A_w_o, B_w1.T, B_w2)
```

```python
import jax
import jax.numpy as jnp
from jax import lax
from jax.experimental import pallas as pl
from jax.experimental.pallas import tpu as pltpu

F32 = jnp.float32
BF16 = jnp.bfloat16
I32 = jnp.int32
_NN = (((1,), (0,)), ((), ()))
_NT = (((1,), (1,)), ((), ()))
LANES = 128

_KEY_BLOCK = 1024
_CKV_PIECES = (16, 9, 5, 2)
_WO_PIECES = (16, 8, 4, 2, 1, 1)
_WO_GROUP = 4
_IN_FLIGHT = 3


def _dot(a, b, dims=_NN):
    return lax.dot_general(a, b, dims, preferred_element_type=F32)


def _pieces(sizes):
    out, start = [], 0
    for n in sizes:
        out.append((start, n))
        start += n
    return out


def _split(total, sizes):
    return tuple(sizes) if sum(sizes) == total else (total,)


def _kernel(x_h, c_h, wq_h, wk_h, wv_h, wo_h, w1t_h, w2_h, o_ref,
            x_v, c_v, wq_v, wk_v, wv_v, wo_v, w1t_v, w2_v,
            xn_v, qa_v, y_v, lhs_v, sems):
    M, H, D = wq_h.shape
    DC = wk_h.shape[0]
    SK = c_h.shape[1]
    BK = _KEY_BLOCK
    c_pieces = _pieces(_split(SK // BK, _CKV_PIECES))
    wo_pieces = _pieces(_split(H, _WO_PIECES))
    G = LANES // H

    copies = [(x_h, x_v), (w1t_h, w1t_v), (w2_h, w2_v), (wq_h, wq_v), (wk_h, wk_v)]
    copies += [(c_h.at[0, pl.ds(s * BK, n * BK)], c_v.at[pl.ds(s * BK, n * BK)])
               for s, n in c_pieces]
    copies += [(wv_h, wv_v)]
    copies += [(wo_h.at[pl.ds(s, n)], wo_v.at[pl.ds(s, n)]) for s, n in wo_pieces]
    dmas = [pltpu.make_async_copy(src, dst, sems.at[i % _IN_FLIGHT])
            for i, (src, dst) in enumerate(copies)]
    for dma in dmas[:_IN_FLIGHT]:
        dma.start()
    arrived = []

    def wait_next():
        i = len(arrived)
        dmas[i].wait()
        arrived.append(i)
        if i + _IN_FLIGHT < len(dmas):
            dmas[i + _IN_FLIGHT].start()

    wait_next()
    x = x_v[0].astype(F32)
    xc = x - jnp.mean(x, axis=-1, keepdims=True)
    var = jnp.mean(xc * xc, axis=-1, keepdims=True)
    xn = xc / jnp.sqrt(var + 1e-5)
    xn_v[...] = jnp.broadcast_to(xn, xn_v.shape)

    xb = jnp.broadcast_to(xn, (16, M)).astype(BF16)
    wait_next()
    h1 = _dot(xb, w1t_v[...], _NT)
    h1 = h1 * jax.nn.sigmoid(h1)
    wait_next()
    ff = _dot(h1.astype(BF16), w2_v[...])[0:1]
    gate = ff * jax.nn.sigmoid(ff)

    row = lax.broadcasted_iota(I32, (H, LANES), 0)
    lane = lax.broadcasted_iota(I32, (H, LANES), 1)
    spread = lane // H
    diag = (lane % H) == row

    def per_head_matvec(y, w_ref, c0):
        parts = []
        for u in range(LANES // G):
            g = jnp.take_along_axis(y, G * u + spread, axis=1)
            parts.append(jnp.where(diag, g, 0.0).astype(BF16))
        s = jnp.concatenate(parts, axis=1)
        return _dot(s, w_ref[pl.ds(c0, LANES)].reshape(LANES * H, D))

    wait_next()

    def q_step(t, q):
        m0 = pl.multiple_of(t * LANES, LANES)
        y = jnp.broadcast_to(xn_v[0:1, pl.ds(m0, LANES)], (H, LANES))
        return q + per_head_matvec(y, wq_v, m0)

    zero = jnp.zeros((H, D), F32)
    q = lax.fori_loop(0, M // LANES, q_step, zero).astype(BF16)

    wait_next()
    pick = (lane % G) * H + row

    def qabs_step(t, carry):
        c0 = pl.multiple_of(t * LANES, LANES)
        r = _dot(q, wk_v[pl.ds(c0, LANES)].reshape(LANES * H, D), _NT)
        out = jnp.zeros((H, LANES), F32)
        for u in range(LANES // G):
            g = jnp.take_along_axis(r[:, u * LANES:(u + 1) * LANES], pick, axis=1)
            out = jnp.where(lane // G == u, g, out)
        qa_v[:, pl.ds(c0, LANES)] = (out * (D ** -0.5)).astype(BF16)
        return carry

    lax.fori_loop(0, DC // LANES, qabs_step, 0)

    def attend(block, carry):
        m_run, l_run, acc = carry
        cb = c_v[pl.ds(pl.multiple_of(block * BK, BK), BK), :]
        s = _dot(qa_v[...], cb, _NT)
        m_new = jnp.maximum(m_run, jnp.max(s, axis=1, keepdims=True))
        alpha = jnp.exp(m_run - m_new)
        p = jnp.exp(s - m_new)
        l_run = alpha * l_run + jnp.sum(p, axis=1, keepdims=True)
        acc = alpha * acc + _dot(p.astype(BF16), cb)
        return m_new, l_run, acc

    carry = (jnp.full((H, 1), -jnp.inf, F32), jnp.zeros((H, 1), F32), jnp.zeros((H, DC), F32))
    for s0, n in c_pieces:
        wait_next()
        carry = lax.fori_loop(s0, s0 + n, attend, carry)
    _, l_run, acc = carry
    y_v[...] = acc / l_run

    wait_next()

    def ctx_step(t, ctx):
        c0 = pl.multiple_of(t * LANES, LANES)
        return ctx + per_head_matvec(y_v[:, pl.ds(c0, LANES)], wv_v, c0)

    ctx = lax.fori_loop(0, DC // LANES, ctx_step, zero)

    for h in range(H):
        lhs_v[:, h * D:(h + 1) * D] = jnp.broadcast_to(ctx[h:h + 1], (16, D)).astype(BF16)

    def heads(h0, n):
        return _dot(lhs_v[:, pl.ds(pl.multiple_of(h0 * D, D), n * D)],
                    wo_v[pl.ds(h0, n)].reshape(n * D, M))

    o = jnp.zeros((16, M), F32)
    U = _WO_GROUP
    for s0, n in wo_pieces:
        wait_next()
        if n // U > 1:
            o = lax.fori_loop(0, n // U, lambda j, o, s0=s0: o + heads(s0 + j * U, U), o)
        elif n // U == 1:
            o = o + heads(s0, U)
        if n % U:
            o = o + heads(s0 + n // U * U, n % U)
    o_ref[0] = (x + o[0:1] * gate).astype(o_ref.dtype)


@jax.jit
def pallas_recurrent_scan__compressed_kv_cla__dense_activation_silu__decode_kernel(
    A_x: jax.Array,
    A_c_kv: jax.Array,
    A_w_q: jax.Array,
    A_w_uk: jax.Array,
    A_w_uv: jax.Array,
    A_w_o: jax.Array,
    B_x: jax.Array,
    B_w1: jax.Array,
    B_w2: jax.Array,
):
    del B_x
    B, Sq, M = A_x.shape
    _, SK, DC = A_c_kv.shape
    _, H, D = A_w_q.shape
    FF = B_w1.shape[1]
    assert B == 1 and Sq == 1 and D == LANES and LANES % H == 0 and DC % LANES == 0
    assert SK % _KEY_BLOCK == 0 and M % LANES == 0

    return pl.pallas_call(
        _kernel,
        out_shape=jax.ShapeDtypeStruct(A_x.shape, A_x.dtype),
        in_specs=[pl.BlockSpec(memory_space=pl.ANY)] * 8,
        out_specs=pl.BlockSpec(memory_space=pltpu.VMEM),
        scratch_shapes=[
            pltpu.VMEM((B, Sq, M), A_x.dtype),
            pltpu.VMEM((SK, DC), A_c_kv.dtype),
            pltpu.VMEM(A_w_q.shape, A_w_q.dtype),
            pltpu.VMEM(A_w_uk.shape, A_w_uk.dtype),
            pltpu.VMEM(A_w_uv.shape, A_w_uv.dtype),
            pltpu.VMEM(A_w_o.shape, A_w_o.dtype),
            pltpu.VMEM((FF, M), B_w1.dtype),
            pltpu.VMEM((FF, M), B_w2.dtype),
            pltpu.VMEM((8, M), F32),
            pltpu.VMEM((H, DC), BF16),
            pltpu.VMEM((H, DC), F32),
            pltpu.VMEM((16, H * D), BF16),
            pltpu.SemaphoreType.DMA((_IN_FLIGHT,)),
        ],
        compiler_params=pltpu.CompilerParams(vmem_limit_bytes=100 * 1024 * 1024),
    )(A_x, A_c_kv, A_w_q, A_w_uk, A_w_uv, A_w_o, B_w1.T, B_w2)
```

```python
import jax
import jax.numpy as jnp
from jax import lax
from jax.experimental import pallas as pl
from jax.experimental.pallas import tpu as pltpu

F32 = jnp.float32
BF16 = jnp.bfloat16
I32 = jnp.int32
_NN = (((1,), (0,)), ((), ()))
_NT = (((1,), (1,)), ((), ()))
LANES = 128

_KEY_BLOCK = 1024
_BLOCKS_PER_COPY = 4
_WO_STEP = 512
_WO_MXU_PIECES = (1024, 1024, 1024, 512)
_WO_VPU_PIECES = (256, 128, 64, 32, 16, 16)


def _dot(a, b, dims=_NN):
    return lax.dot_general(a, b, dims, preferred_element_type=F32)


def _pieces(sizes, start=0):
    out = []
    for n in sizes:
        out.append((start, n))
        start += n
    return out


def _wo_pieces(rows):
    if sum(_WO_MXU_PIECES) + sum(_WO_VPU_PIECES) == rows:
        return _pieces(_WO_MXU_PIECES), _pieces(_WO_VPU_PIECES, sum(_WO_MXU_PIECES))
    return _pieces((rows - LANES,)), _pieces((LANES,), rows - LANES)


def _decode_step(x_h, c_h, wq_h, wk_h, wv_h, wo_h, w1t_h, w2_h, o_ref,
                 x_v, c_v, wq_v, wk_v, wv_v, wo_v, w1t_v, w2_v,
                 xn_v, qa_v, y_v, lhs_v, col_v, sems):
    M, H, D = wq_h.shape
    DC = wk_h.shape[0]
    SK = c_h.shape[1]
    BK, PB = _KEY_BLOCK, _BLOCKS_PER_COPY
    G = LANES // H
    mxu_pieces, vpu_pieces = _wo_pieces(H * D)

    def cache_copy(i, sem):
        rows = pl.ds(pl.multiple_of(i * (PB * BK), PB * BK), PB * BK)
        return pltpu.make_async_copy(c_h.at[0, rows], c_v.at[rows], sem)

    n_cache = SK // (PB * BK)
    head = [(x_h, x_v), (w1t_h, w1t_v), (w2_h, w2_v), (wq_h, wq_v), (wk_h, wk_v)]
    tail = [(wv_h, wv_v)]
    tail += [(wo_h.at[pl.ds(s, n)], wo_v.at[pl.ds(s, n)]) for s, n in mxu_pieces + vpu_pieces]
    dmas = [pltpu.make_async_copy(src, dst, sems.at[i]) for i, (src, dst) in enumerate(head)]
    dmas += [cache_copy(i, sems.at[len(head) + i]) for i in range(n_cache)]
    dmas += [pltpu.make_async_copy(src, dst, sems.at[len(head) + n_cache + i])
             for i, (src, dst) in enumerate(tail)]
    for dma in dmas:
        dma.start()
    todo = iter(dmas[:len(head)] + dmas[len(head) + n_cache:])

    def wait_next():
        next(todo).wait()

    wait_next()
    x = x_v[0].astype(F32)
    xc = x - jnp.mean(x, axis=-1, keepdims=True)
    var = jnp.mean(xc * xc, axis=-1, keepdims=True)
    xn = xc / jnp.sqrt(var + 1e-5)
    xn_v[...] = jnp.broadcast_to(xn, xn_v.shape)

    xb = jnp.broadcast_to(xn, (16, M)).astype(BF16)
    wait_next()
    h1 = _dot(xb, w1t_v[...], _NT)
    h1 = h1 * jax.nn.sigmoid(h1)
    wait_next()
    ff = _dot(h1.astype(BF16), w2_v[...])[0:1]
    gate = ff * jax.nn.sigmoid(ff)

    row = lax.broadcasted_iota(I32, (H, LANES), 0)
    lane = lax.broadcasted_iota(I32, (H, LANES), 1)
    spread = lane // H
    diag = (lane % H) == row

    def per_head_matvec(y, w_ref, c0):
        parts = []
        for u in range(LANES // G):
            g = jnp.take_along_axis(y, G * u + spread, axis=1)
            parts.append(jnp.where(diag, g, 0.0).astype(BF16))
        s = jnp.concatenate(parts, axis=1)
        return _dot(s, w_ref[pl.ds(c0, LANES)].reshape(LANES * H, D))

    wait_next()

    def q_step(t, q):
        m0 = pl.multiple_of(t * LANES, LANES)
        y = jnp.broadcast_to(xn_v[0:1, pl.ds(m0, LANES)], (H, LANES))
        return q + per_head_matvec(y, wq_v, m0)

    zero = jnp.zeros((H, D), F32)
    q = lax.fori_loop(0, M // LANES, q_step, zero).astype(BF16)

    wait_next()
    pick = (lane % G) * H + row

    def qabs_step(t, carry):
        c0 = pl.multiple_of(t * LANES, LANES)
        r = _dot(q, wk_v[pl.ds(c0, LANES)].reshape(LANES * H, D), _NT)
        out = jnp.zeros((H, LANES), F32)
        for u in range(LANES // G):
            g = jnp.take_along_axis(r[:, u * LANES:(u + 1) * LANES], pick, axis=1)
            out = jnp.where(lane // G == u, g, out)
        qa_v[:, pl.ds(c0, LANES)] = (out * (D ** -0.5)).astype(BF16)
        return carry

    lax.fori_loop(0, DC // LANES, qabs_step, 0)

    def attend(block, carry):
        @pl.when(block % PB == 0)
        def _():
            cache_copy(block // PB, sems.at[len(head) + block // PB]).wait()

        m_run, l_run, acc = carry
        cb = c_v[pl.ds(pl.multiple_of(block * BK, BK), BK), :]
        s = _dot(qa_v[...], cb, _NT)
        m_new = jnp.maximum(m_run, jnp.max(s, axis=1, keepdims=True))
        alpha = jnp.exp(m_run - m_new)
        p = jnp.exp(s - m_new)
        l_run = alpha * l_run + jnp.sum(p, axis=1, keepdims=True)
        acc = alpha * acc + _dot(p.astype(BF16), cb)
        return m_new, l_run, acc

    carry = (jnp.full((H, 1), -jnp.inf, F32), jnp.zeros((H, 1), F32), jnp.zeros((H, DC), F32))
    _, l_run, acc = lax.fori_loop(0, SK // BK, attend, carry)
    y_v[...] = acc / l_run

    wait_next()

    def ctx_step(t, ctx):
        c0 = pl.multiple_of(t * LANES, LANES)
        return ctx + per_head_matvec(y_v[:, pl.ds(c0, LANES)], wv_v, c0)

    ctx = lax.fori_loop(0, DC // LANES, ctx_step, zero)

    r_vpu = vpu_pieces[0][0]
    for h in range(pl.cdiv(r_vpu, D)):
        lhs_v[:, h * D:(h + 1) * D] = jnp.broadcast_to(ctx[h:h + 1], (16, D)).astype(BF16)
    h_vpu = r_vpu // D
    dd = lax.broadcasted_iota(I32, (D, LANES), 0)
    ll = lax.broadcasted_iota(I32, (D, LANES), 1)
    for h in range(h_vpu, H):
        col = jnp.sum(jnp.where(dd == ll, jnp.broadcast_to(ctx[h:h + 1], (D, LANES)), 0.0),
                      axis=1, keepdims=True)
        col_v[pl.ds((h - h_vpu) * D, D), :] = jnp.broadcast_to(col, (D, LANES))

    def project(r0, n):
        return _dot(lhs_v[:, pl.ds(r0, n)], wo_v[pl.ds(r0, n), :])

    o = jnp.zeros((16, M), F32)
    for s0, n in mxu_pieces:
        wait_next()
        steps = n // _WO_STEP
        if steps > 1:
            o = lax.fori_loop(
                0, steps,
                lambda j, o, s0=s0: o + project(pl.multiple_of(s0 + j * _WO_STEP, LANES), _WO_STEP),
                o)
        elif steps == 1:
            o = o + project(s0, _WO_STEP)
        if n % _WO_STEP:
            o = o + project(s0 + steps * _WO_STEP, n % _WO_STEP)
    res = x + o[0:1] * gate

    part = [jnp.zeros((8, LANES), F32) for _ in range(M // LANES)]
    for s0, n in vpu_pieces:
        wait_next()
        w = wo_v[pl.ds(s0, n), :].astype(F32)
        cv = col_v[pl.ds(s0 - h_vpu * D, n), :]
        for j in range(M // LANES):
            prod = w[:, j * LANES:(j + 1) * LANES] * cv
            part[j] = part[j] + jnp.sum(prod.reshape(n // 8, 8, LANES), axis=0)
    rest = jnp.concatenate([jnp.sum(a, axis=0, keepdims=True) for a in part], axis=1)
    o_ref[0] = (res + rest * gate).astype(o_ref.dtype)


def _kernel(*refs, n_copies):
    pl.run_scoped(lambda sems: _decode_step(*refs, sems), pltpu.SemaphoreType.DMA((n_copies,)))


@jax.jit
def pallas_recurrent_scan__compressed_kv_cla__dense_activation_silu__decode_kernel(
    A_x: jax.Array,
    A_c_kv: jax.Array,
    A_w_q: jax.Array,
    A_w_uk: jax.Array,
    A_w_uv: jax.Array,
    A_w_o: jax.Array,
    B_x: jax.Array,
    B_w1: jax.Array,
    B_w2: jax.Array,
):
    del B_x
    B, Sq, M = A_x.shape
    _, SK, DC = A_c_kv.shape
    _, H, D = A_w_q.shape
    FF = B_w1.shape[1]
    assert B == 1 and Sq == 1 and D == LANES and LANES % H == 0
    assert M % LANES == 0 and DC % LANES == 0 and SK % (_KEY_BLOCK * _BLOCKS_PER_COPY) == 0
    mxu_pieces, vpu_pieces = _wo_pieces(H * D)
    n_copies = 6 + SK // (_KEY_BLOCK * _BLOCKS_PER_COPY) + len(mxu_pieces) + len(vpu_pieces)
    mxu_rows = pl.cdiv(vpu_pieces[0][0], D) * D
    vpu_rows = H * D - vpu_pieces[0][0] // D * D

    return pl.pallas_call(
        lambda *refs: _kernel(*refs, n_copies=n_copies),
        out_shape=jax.ShapeDtypeStruct(A_x.shape, A_x.dtype),
        in_specs=[pl.BlockSpec(memory_space=pl.ANY)] * 8,
        out_specs=pl.BlockSpec(memory_space=pltpu.VMEM),
        scratch_shapes=[
            pltpu.VMEM((B, Sq, M), A_x.dtype),
            pltpu.VMEM((SK, DC), A_c_kv.dtype),
            pltpu.VMEM(A_w_q.shape, A_w_q.dtype),
            pltpu.VMEM(A_w_uk.shape, A_w_uk.dtype),
            pltpu.VMEM(A_w_uv.shape, A_w_uv.dtype),
            pltpu.VMEM((H * D, M), A_w_o.dtype),
            pltpu.VMEM((FF, M), B_w1.dtype),
            pltpu.VMEM((FF, M), B_w2.dtype),
            pltpu.VMEM((8, M), F32),
            pltpu.VMEM((H, DC), BF16),
            pltpu.VMEM((H, DC), F32),
            pltpu.VMEM((16, mxu_rows), BF16),
            pltpu.VMEM((vpu_rows, LANES), F32),
        ],
        compiler_params=pltpu.CompilerParams(vmem_limit_bytes=100 * 1024 * 1024),
        name="mla_decode_step",
    )(A_x, A_c_kv, A_w_q, A_w_uk, A_w_uv, A_w_o.reshape(H * D, M), B_w1.T, B_w2)
```
